```python
import os as _os
_os.environ.setdefault("JAX_PLATFORMS", "cpu")
import jax
import jax.numpy as jnp

def _softmax(x, axis=-1):
    return jax.nn.softmax(x, axis=axis)
def _gelu(x):
    return jax.nn.gelu(x, approximate=True)
def _silu(x):
    return jax.nn.silu(x)
def _sigmoid(x):
    return jax.nn.sigmoid(x)
def _layernorm(x, axis=-1, eps=1e-5):
    m = jnp.mean(x, axis=axis, keepdims=True)
    v = jnp.var(x, axis=axis, keepdims=True)
    return (x - m) / jnp.sqrt(v + eps)
def _scatter_add(tgt, idx, src, axis=0):
    return tgt.at[idx].add(src)
def _segment_sum(src, seg, n):
    return jax.ops.segment_sum(src, seg, n)
class _Rng:
    def __init__(self, key):
        self._k = key
    def _next(self):
        self._k, sub = jax.random.split(self._k)
        return sub
    def normal(self, shape):
        return jax.random.normal(self._next(), shape, dtype=jnp.bfloat16)
    def randint(self, lo, hi, shape):
        return jax.random.randint(self._next(), shape, lo, hi, dtype=jnp.int32)
    def uniform(self, shape, lo=0.0, hi=1.0):
        return jax.random.uniform(self._next(), shape, jnp.bfloat16, lo, hi)
    def permutation(self, n):
        return jax.random.permutation(self._next(), n)


kernel_name = 'sequential_preLN__softmax_full_mha__dense_activation_squared_relu__prompt'

def setup_inputs():
    _rng = _Rng(jax.random.key(int.from_bytes(__import__("os").urandom(4), "little")))
    _w = (lambda a: (lambda t: t.astype(jnp.bfloat16) if jnp.issubdtype(t.dtype, jnp.floating) else t)(jnp.asarray(a)))
    def _A_setup():
        B, S, D = 1, 2048, 640
        return {
            "x": _w((lambda *s: _rng.normal(s) * 0.05)(B, S, D)),
            "wqkv": _w((lambda *s: _rng.normal(s) * 0.05)(D, 3 * D)),
            "wo": _w((lambda *s: _rng.normal(s) * 0.05)(D, D)),
        }
    _A_in = _A_setup()

    def _B_setup():
        B, S, D, F = 1, 2048, 640, 1536
        return {
            "x": _w((lambda *s: _rng.normal(s) * 0.05)(B, S, D)),
            "w1": _w((lambda *s: _rng.normal(s) * 0.05)(D, F)),
            "b1": _w((lambda *s: _rng.normal(s) * 0.05)(F)),
            "w2": _w((lambda *s: _rng.normal(s) * 0.05)(F, D)),
            "b2": _w((lambda *s: _rng.normal(s) * 0.05)(D)),
        }
    _B_in = _B_setup()

    return {
        "A_x": _A_in["x"],
        "A_wqkv": _A_in["wqkv"],
        "A_wo": _A_in["wo"],
        "B_x": _B_in["x"],
        "B_w1": _B_in["w1"],
        "B_b1": _B_in["b1"],
        "B_w2": _B_in["w2"],
        "B_b2": _B_in["b2"],
    }

def reference(A_x, A_wqkv, A_wo, B_x, B_w1, B_b1, B_w2, B_b2):
    def _A_ref(x, wqkv, wo):
        B, S, D = x.shape
        H = 32; Dh = D // H
        qkv = (lambda x, *d: x.transpose(*d))((x @ wqkv).reshape(B, S, 3, H, Dh), 2, 0, 3, 1, 4)
        q, k, v = qkv[0], qkv[1], qkv[2]
        scale = Dh ** -0.5
        scores = jnp.einsum("bhqd,bhkd->bhqk", q, k) * scale
        p = _softmax(scores, axis=-1)
        o = jnp.einsum("bhqk,bhkd->bhqd", p, v)
        return (lambda x, *d: x.transpose(*d))(o, 0, 2, 1, 3).reshape(B, S, D) @ wo

    def _B_ref(x, w1, b1, w2, b2):
        h = jnp.einsum("bsd,df->bsf", x, w1) + b1
        zero = jnp.zeros_like(h)
        r = jnp.where(h > zero, h, zero)
        h = r * r
        out = jnp.einsum("bsf,fd->bsd", h, w2) + b2
        return out

    x = A_x
    h = x + _A_ref(_layernorm(x, axis=-1), A_wqkv, A_wo)
    h2 = h + _B_ref(_layernorm(h, axis=-1), B_w1, B_b1, B_w2, B_b2)
    return h2
```

```python
import functools
import math

import jax
import jax.numpy as jnp
from jax import lax
import jax.experimental.pallas as pl
import jax.experimental.pallas.tpu as pltpu

BF16 = jnp.bfloat16
F32 = jnp.float32

NUM_HEADS = 32
LN_EPS = 1e-5
LANES = 128

CFG = dict(NQ=512, CH=128, RB=512, FB=512, PAIRS=1)


def _dot(a, b):
    return jnp.dot(a, b, preferred_element_type=F32)


def _dot_nt(a, b):
    return lax.dot_general(a, b, (((1,), (1,)), ((), ())), preferred_element_type=F32)


def _layernorm(x):
    mean = jnp.mean(x, axis=-1, keepdims=True)
    xc = x - mean
    var = jnp.mean(xc * xc, axis=-1, keepdims=True)
    return xc * lax.rsqrt(var + LN_EPS)


def _kernel(x_hbm, wqkv_hbm, wo_hbm, w1_hbm, b1_hbm, w2_hbm, b2_hbm, out_hbm,
            x_s, wqkv_s, wo_s, w1_s, b1_s, w2_s, b2_s,
            wqt_s, wvt_s, k_s, qt_s, vt_s, s_s, ot_s, out_s, in_sem, out_sem, *, cfg):
    S, D = x_s.shape
    H = NUM_HEADS
    DH = D // H
    NQ, CH, RB, FB = cfg["NQ"], cfg["CH"], cfg["RB"], cfg["FB"]
    NSLAB = D // LANES
    NPAIR = H // 2
    q_scale = (DH ** -0.5) * math.log2(math.e)

    n_rb = S // RB
    x_cp = [pltpu.make_async_copy(x_hbm.at[0, pl.ds(r * RB, RB), :], x_s.at[pl.ds(r * RB, RB), :], in_sem.at[r])
            for r in range(n_rb)]
    others = [(wqkv_hbm, wqkv_s), (wo_hbm, wo_s), (w1_hbm, w1_s), (b1_hbm, b1_s), (w2_hbm, w2_s), (b2_hbm, b2_s)]
    w_cp = [pltpu.make_async_copy(src, dst, in_sem.at[n_rb + i]) for i, (src, dst) in enumerate(others)]
    x_cp[0].start()
    w_cp[0].start()
    for c in x_cp[1:]:
        c.start()
    for c in w_cp[1:]:
        c.start()

    w_cp[0].wait()
    wqt_s[...] = wqkv_s[:, 0:D].T
    wvt_s[...] = wqkv_s[:, 2 * D:3 * D].T
    lane = lax.broadcasted_iota(jnp.int32, (RB, LANES), 1)
    row8 = lax.broadcasted_iota(jnp.int32, (8, RB), 0)
    for r in range(n_rb):
        rows = pl.ds(r * RB, RB)
        x_cp[r].wait()
        ln = _layernorm(x_s[rows, :].astype(F32)).astype(BF16)
        k = _dot(ln, wqkv_s[:, D:2 * D])
        slabs = [k[:, j * LANES:(j + 1) * LANES] for j in range(NSLAB)]
        for j in range(NSLAB):
            k_s[2 * j, rows, :] = slabs[j].astype(BF16)
            if j + 1 < NSLAB:
                k_s[2 * j + 1, rows, :] = jnp.where(lane >= LANES // 2, slabs[j], slabs[j + 1]).astype(BF16)
        qt_s[:, rows] = _dot_nt(wqt_s[...], ln) * q_scale
        vt = _dot_nt(wvt_s[...], ln).astype(BF16).astype(F32)
        for p in range(NPAIR):
            b = 2 * DH * p
            mid = vt[b + 16:b + 24]
            vt_s[p, 0:16, rows] = vt[b:b + 16]
            vt_s[p, 16:24, rows] = jnp.where(row8 < 4, mid, 1.0)
            vt_s[p, 24:32, rows] = jnp.where(row8 >= 4, mid, 1.0)
            vt_s[p, 32:48, rows] = vt[b + 24:b + 40]

    n_qb = S // NQ
    NC = S // CH
    qrow = lax.broadcasted_iota(jnp.int32, (LANES, NQ), 0)

    def q_weights(h, qcols):
        lo = h * DH
        j = lo // LANES
        straddle = ((lo + DH - 1) // LANES > j).astype(jnp.int32) if not isinstance(h, int) else int((lo + DH - 1) // LANES > j)
        half = LANES // 2
        top = pl.multiple_of((j + straddle) * LANES, half) if not isinstance(h, int) else (j + straddle) * LANES
        bot = pl.multiple_of(j * LANES + half, half) if not isinstance(h, int) else j * LANES + half
        q = jnp.concatenate([qt_s[pl.ds(top, half), qcols], qt_s[pl.ds(bot, half), qcols]], axis=0)
        col = qrow + jnp.where(qrow < half, (j + straddle) * LANES, j * LANES)
        q = jnp.where((col >= lo) & (col < lo + DH), q, 0.0).astype(BF16)
        return q, 2 * j + straddle

    def half_step(scores, values):
        m = acc = None
        if scores is not None:
            h, qcols, slot = scores
            q, slab = q_weights(h, qcols)
        for c in range(NC):
            keys = pl.ds(c * CH, CH)
            if scores is not None:
                s = _dot(k_s[slab, keys, :], q)
                s_s[slot, keys, :] = s
                cm = jnp.max(s.reshape(CH // 8, 8, NQ), axis=0)
                m = cm if m is None else jnp.maximum(m, cm)
            if values is not None:
                pair, parity, vslot, vm = values
                p = jnp.exp2(s_s[vslot, keys, :] - vm).astype(BF16)
                o = _dot(vt_s[pair, pl.ds(24 * parity, 24), keys], p)
                acc = o if acc is None else acc + o
        if m is not None:
            m = jnp.max(m, axis=0, keepdims=True)
        return m, acc

    row8q = lax.broadcasted_iota(jnp.int32, (8, NQ), 0)

    def finish(pair, qcols, acc_e, acc_o):
        inv_e = 1.0 / acc_e[20:21]
        inv_o = 1.0 / acc_o[0:1]
        base = pair * (2 * DH)
        if not isinstance(base, int):
            base = pl.multiple_of(base, 8)
        ot_s[pl.ds(base, 16), qcols] = acc_e[0:16] * inv_e
        ot_s[pl.ds(base + 16, 8), qcols] = jnp.where(row8q < 4, acc_e[16:24] * inv_e, acc_o[0:8] * inv_o)
        ot_s[pl.ds(base + 24, 16), qcols] = acc_o[8:24] * inv_o

    def qcols_of(item):
        return pl.ds(pl.multiple_of((item // NPAIR) * NQ, NQ), NQ)

    n_items = n_qb * NPAIR
    m0, _ = half_step((0, pl.ds(0, NQ), 0), None)

    def item_body(i, m_e):
        pair = i % NPAIR
        qcols = qcols_of(i)
        m_o, acc_e = half_step((2 * pair + 1, qcols, 1), (pair, 0, 0, m_e))
        nxt = i + 1
        m_n, acc_o = half_step((2 * (nxt % NPAIR), qcols_of(nxt), 0), (pair, 1, 1, m_o))
        finish(pair, qcols, acc_e, acc_o)
        return m_n

    m_e = lax.fori_loop(0, n_items - 1, item_body, m0)
    last_cols = pl.ds(S - NQ, NQ)
    m_o, acc_e = half_step((H - 1, last_cols, 1), (NPAIR - 1, 0, 0, m_e))
    _, acc_o = half_step(None, (NPAIR - 1, 1, 1, m_o))
    finish(NPAIR - 1, last_cols, acc_e, acc_o)

    for c in w_cp[1:]:
        c.wait()
    b1 = b1_s[...].astype(F32).reshape(1, -1)
    b2 = b2_s[...].astype(F32).reshape(1, -1)
    n_fb = S // FB
    out_cp = []
    for r in range(n_fb):
        rows = pl.ds(r * FB, FB)
        o = ot_s[:, rows].T.astype(BF16)
        h = x_s[rows, :].astype(F32) + _dot(o, wo_s[...])
        ln = _layernorm(h).astype(BF16)
        a = jnp.maximum(_dot(ln, w1_s[...]) + b1, 0.0)
        y = _dot((a * a).astype(BF16), w2_s[...]) + b2
        out_s[rows, :] = (h + y).astype(out_s.dtype)
        cp = pltpu.make_async_copy(out_s.at[rows, :], out_hbm.at[0, rows, :], out_sem.at[r])
        cp.start()
        out_cp.append(cp)
    for cp in out_cp:
        cp.wait()


def build(cfg):
    def fn(A_x, A_wqkv, A_wo, B_x, B_w1, B_b1, B_w2, B_b2):
        del B_x
        _, S, D = A_x.shape
        F = B_w1.shape[1]
        NQ = cfg["NQ"]
        hbm = pl.BlockSpec(memory_space=pl.ANY)
        n_slab = 2 * (D // LANES) - 1
        scratch = [
            pltpu.VMEM((S, D), A_x.dtype),
            pltpu.VMEM(A_wqkv.shape, A_wqkv.dtype),
            pltpu.VMEM(A_wo.shape, A_wo.dtype),
            pltpu.VMEM(B_w1.shape, B_w1.dtype),
            pltpu.VMEM(B_b1.shape, B_b1.dtype),
            pltpu.VMEM(B_w2.shape, B_w2.dtype),
            pltpu.VMEM(B_b2.shape, B_b2.dtype),
            pltpu.VMEM((D, D), BF16),
            pltpu.VMEM((D, D), BF16),
            pltpu.VMEM((n_slab, S, LANES), BF16),
            pltpu.VMEM((D, S), F32),
            pltpu.VMEM((NUM_HEADS // 2, 48, S), F32),
            pltpu.VMEM((2, S, NQ), F32),
            pltpu.VMEM((D, S), F32),
            pltpu.VMEM((S, D), A_x.dtype),
            pltpu.SemaphoreType.DMA((S // cfg["RB"] + 6,)),
            pltpu.SemaphoreType.DMA((S // cfg["FB"],)),
        ]
        return pl.pallas_call(
            functools.partial(_kernel, cfg=cfg),
            out_shape=jax.ShapeDtypeStruct(A_x.shape, A_x.dtype),
            in_specs=[hbm] * 7,
            out_specs=hbm,
            scratch_shapes=scratch,
            compiler_params=pltpu.CompilerParams(vmem_limit_bytes=110 * 2**20, flags=cfg.get("flags")),
        )(A_x, A_wqkv, A_wo, B_w1, B_b1, B_w2, B_b2)
    return fn


@jax.jit
def pallas_sequential_preLN__softmax_full_mha__dense_activation_squared_relu__prompt_kernel(
    A_x: jax.Array,
    A_wqkv: jax.Array,
    A_wo: jax.Array,
    B_x: jax.Array,
    B_w1: jax.Array,
    B_b1: jax.Array,
    B_w2: jax.Array,
    B_b2: jax.Array,
):
    return build(CFG)(A_x, A_wqkv, A_wo, B_x, B_w1, B_b1, B_w2, B_b2)
```

```python
import functools
import math

import jax
import jax.numpy as jnp
from jax import lax
import jax.experimental.pallas as pl
import jax.experimental.pallas.tpu as pltpu

BF16 = jnp.bfloat16
F32 = jnp.float32
U32 = jnp.uint32

NUM_HEADS = 32
LN_EPS = 1e-5
LANES = 128
NQ = 512
CH = 128
NV = 16
HROWS = 24
SUM_LO, SUM_HI, VALUE_HI = 2.0 ** -20, 2.0 ** 90, 2.0 ** 36

CFG = dict(flip=0, qstart=0, dyn="pkq", small=128, big=256, p1="0c1d23", klay=1, play=1, loop1=0, loop3=1, kfirst=1, RB=512, FB=256, pos="2,3,4,5,6", qmode="iter", nmk=10, qanch=1, kanch=1)


def _dot(a, b):
    return jnp.dot(a, b, preferred_element_type=F32)


def _dot_nt(a, b):
    return lax.dot_general(a, b, (((1,), (1,)), ((), ())), preferred_element_type=F32)


def _layernorm(x):
    mean = jnp.mean(x, axis=-1, keepdims=True)
    xc = x - mean
    var = jnp.mean(xc * xc, axis=-1, keepdims=True)
    return xc * lax.rsqrt(var + LN_EPS)


def _kernel(x_hbm, wqkv_hbm, wo_hbm, w1_hbm, b1_hbm, w2_hbm, b2_hbm, out_hbm,
            x_s, wq_s, wk_s, wv_s, wo_s, w1_s, b1_s, w2_s, b2_s,
            ln_s, h_s, k_s, q_s, v_s, p_s, kb_s, qb_s, pv_s, range_s, vmax_s, o_s, out_s, zero_s, in_sem, out_sem, *, cfg):
    S, D = x_s.shape
    H = NUM_HEADS
    DH = D // H
    RB, FB = cfg["RB"], cfg["FB"]
    NSLAB = D // LANES
    NPAIR = H // 2
    NT = NQ // LANES
    NC = S // CH
    NQB = S // NQ
    q_scale = (DH ** -0.5) * math.log2(math.e)

    n_rb = S // RB

    def fetch(i, src, dst):
        return pltpu.make_async_copy(src, dst, in_sem.at[i])

    cp_x0 = fetch(0, x_hbm.at[0, pl.ds(0, RB), :], x_s.at[pl.ds(0, RB), :])
    cp_wk = fetch(1, wqkv_hbm.at[:, pl.ds(D, D)], wk_s)
    cp_wq = fetch(2, wqkv_hbm.at[:, pl.ds(0, D)], wq_s)
    cp_wv = fetch(3, wqkv_hbm.at[:, pl.ds(2 * D, D)], wv_s)
    cp_x1 = fetch(4, x_hbm.at[0, pl.ds(RB, RB), :], x_s.at[pl.ds(RB, RB), :])
    cp_x2 = fetch(10, x_hbm.at[0, pl.ds(2 * RB, S - 2 * RB), :], x_s.at[pl.ds(2 * RB, S - 2 * RB), :])
    cp_late = [fetch(5 + i, src, dst) for i, (src, dst) in enumerate(
        [(wo_hbm, wo_s), (w1_hbm, w1_s), (b1_hbm, b1_s), (w2_hbm, w2_s), (b2_hbm, b2_s)])]
    cp_x0.start()
    cp_wk.start()

    def rows_of(r, n=RB):
        return pl.ds(r * n, n) if isinstance(r, int) else pl.ds(pl.multiple_of(r * n, n), n)

    def normalize(lo, n):
        ln_s[lo:lo + n, :] = _layernorm(x_s[lo:lo + n, :].astype(F32)).astype(BF16)

    def project_k(lo, n):
        lane = lax.broadcasted_iota(jnp.int32, (n // 2, LANES), 1)
        k = _dot(ln_s[lo:lo + n, :], wk_s[...]).astype(BF16)
        slabs = [pltpu.bitcast(k[:, j * LANES:(j + 1) * LANES], U32) for j in range(NSLAB)]
        for pair in range(NPAIR):
            j, off = divmod(pair * 2 * DH, LANES)
            kp = slabs[j]
            if off + 2 * DH > LANES:
                kp = jnp.where(lane >= LANES // 2, kp, slabs[j + 1])
            if off:
                kp = pltpu.roll(kp, LANES - off, 1)
            k_s[pair, lo // 2:(lo + n) // 2, :] = kp

    def put_v(pair, row0, lo, val):
        for j in range(val.shape[1] // CH):
            v_s[pair, lo // CH + j, row0:row0 + val.shape[0], :] = val[:, j * CH:(j + 1) * CH]

    def project_qv(lo, n):
        row = lax.broadcasted_iota(jnp.int32, (8, n), 0)
        ln = ln_s[lo:lo + n, :]
        q_s[:, lo:lo + n] = (_dot(ln, wq_s[...]) * q_scale).T
        vt = _dot(ln, wv_s[...]).astype(BF16).astype(F32).T
        vmax = jnp.max(jnp.abs(vt).reshape(D // 8, 8, n), axis=0)
        for j in range(n // LANES):
            vmax_s[...] = jnp.maximum(vmax_s[...], vmax[:, j * LANES:(j + 1) * LANES])
        for pair in range(NPAIR):
            top = pair * 2 * DH
            mid = vt[top + 16:top + 24]
            put_v(pair, 0, lo, vt[top:top + 16])
            put_v(pair, 16, lo, jnp.where(row < 4, mid, 1.0))
            put_v(pair, 24, lo, jnp.where(row >= 4, mid, 1.0))
            put_v(pair, 32, lo, vt[top + 24:top + 40])

    small = cfg["small"]
    vmax_s[...] = jnp.zeros(vmax_s.shape, F32)
    cp_x0.wait()
    normalize(0, RB)
    cp_x1.start()
    cp_wq.start()
    cp_wv.start()
    cp_wk.wait()
    for lo in range(0, RB, small):
        project_k(lo, small)
    cp_x2.start()
    cp_x1.wait()
    for lo in range(RB, 2 * RB, small):
        normalize(lo, small)
        project_k(lo, small)
    cp_wq.wait()
    cp_wv.wait()
    cp_x2.wait()
    if cfg.get("stop") == 2:
        return
    for c in cp_late:
        c.start()
    big = cfg["big"]
    for step in cfg["p1"]:
        for lo in range(0, RB, big):
            if step in "0123":
                project_qv(int(step) * RB + lo, big)
            else:
                normalize("abcd".index(step) * RB + lo, big)
                project_k("abcd".index(step) * RB + lo, big)

    zero_s[0] = 0
    dyn = cfg["dyn"]
    p_u = p_s.bitcast(U32)
    zz = dict(p=0, k=0, q=0)
    never = lax.broadcasted_iota(jnp.int32, (8, LANES), 0) > 8 + (q_s[0:8, 0:LANES] > 0).astype(jnp.int32)
    pos = [int(x) for x in cfg["pos"].split(",")]
    n_piece = len(pos) + 1

    def after(x, y):
        if x.dtype != y.dtype:
            y = pltpu.bitcast(y, x.dtype)
        return jnp.where(never, y, x)

    qrow = lax.broadcasted_iota(jnp.int32, (8, NQ), 0)

    def cols_of(qb):
        return pl.ds(qb * NQ, NQ) if isinstance(qb, int) else pl.ds(pl.multiple_of(qb * NQ, NQ), NQ)

    def pair_rows(pair, lo, n):
        start = pair * 2 * DH + lo
        return pl.ds(start if isinstance(start, int) else pl.multiple_of(start, 8), n)

    def q_weights(pair, odd, qb):
        mid = q_s[pair_rows(pair, 16, 8), cols_of(qb)]
        zero = jnp.zeros((8, NQ), F32)
        if odd:
            parts = [zero, zero, jnp.where(qrow >= 4, mid, 0.0), q_s[pair_rows(pair, 24, 16), cols_of(qb)], zero]
        else:
            parts = [q_s[pair_rows(pair, 0, 16), cols_of(qb)], jnp.where(qrow < 4, mid, 0.0), zero]
        return jnp.concatenate(parts, axis=0).astype(BF16)

    def make_kb(pair, odd, c, d0, d1, anchor=None):
        kv = k_s[pair, (c * CH + CH - NV) // 2:(c * CH + CH) // 2, :]
        if anchor is not None:
            kv = after(kv, anchor)
        kv = pltpu.bitcast(kv, BF16).astype(F32)
        for d in range(d0, d1):
            kb_s[zz["k"], odd, c, d] = jnp.broadcast_to(kv[:, odd * DH + d:odd * DH + d + 1], (NV, LANES))

    def make_qb(pair, odd, qb, d0, d1, anchor=None):
        for d in range(d0, d1):
            r = odd * DH + d
            q8 = q_s[pair_rows(pair, r // 8 * 8, 8), cols_of(qb)]
            if anchor is not None:
                q8 = jnp.concatenate([after(q8[:, j * LANES:(j + 1) * LANES], anchor) for j in range(NT)], axis=1)
            qb_s[zz["q"], qb, d] = jnp.broadcast_to(q8[r % 8:r % 8 + 1, :], (8, NQ))

    def store_out(pair, odd, qb, acc):
        o_s[pair, odd * HROWS:(odd + 1) * HROWS, cols_of(qb)] = acc

    def vpu_scores(kslot, qslot, c, on_partial=None):
        s = None
        for piece in range(n_piece):
            for d in range(piece * DH // n_piece, (piece + 1) * DH // n_piece):
                kb = kb_s[zz["k"], kslot, c, d]
                qv = qb_s[zz["q"], qslot, d]
                t = jnp.concatenate([kb] * NT, axis=1) * jnp.concatenate([qv] * (NV // 8), axis=0)
                s = t if s is None else s + t
            if on_partial is not None and piece < len(pos):
                on_partial(pos[piece], s)
        return jnp.exp2(s).astype(BF16)

    def mxu_scores(h, q, slot, c, on_keys=None):
        lo, n = c * CH, CH - NV
        ks = [k_s[h, (lo + i) // 2:(lo + i) // 2 + 8, :] for i in range(0, n, 16)]
        if on_keys is not None:
            on_keys(ks)
        k = pltpu.bitcast(jnp.concatenate(ks, axis=0), BF16)
        return _dot(k[:, :q.shape[0]], q)

    def store_p(slot, c, s):
        e = jnp.exp2(s)
        if cfg["play"]:
            for i in range((CH - NV) // 16):
                for j in range(NT):
                    p_s[zz["p"], slot, c, i, j] = e[16 * i:16 * i + 16, j * LANES:(j + 1) * LANES].astype(BF16)
            return
        for j in range(NT):
            p_s[slot, j, c * (CH - NV):(c + 1) * (CH - NV), :] = e[:, j * LANES:(j + 1) * LANES].astype(BF16)

    for c in range(NC):
        make_kb(0, 0, c, 0, DH)
    for qb in range(NQB):
        make_qb(0, 0, qb, 0, DH)
    q0 = q_weights(0, 0, 0)
    for c in range(NC):
        store_p(0, c, mxu_scores(0, q0, 0, c))
    pv_s[...] = vpu_scores(0, 0, 0)
    range_s[...] = jnp.ones(range_s.shape, F32)

    def head_body(pair, odd):
        p_vpu, sum_lo, sum_hi = pv_s[...], range_s[odd, 0], range_s[odd, 1]
        z = zero_s[0]
        for name in dyn:
            zz[name] = z
        next_pair = jnp.minimum(pair + 1, NPAIR - 1) if odd else pair
        for qb in range(NQB):
            last = qb == NQB - 1
            ahead = (next_pair, 1 - odd, 0) if last else (pair, odd, qb + 1)
            cur, nxt = qb % 2, (qb + 1) % 2
            q = q_weights(*ahead)
            for c in range(NC):
                lookahead = []

                def on_keys(ks):
                    def on_partial(i, s):
                        for r0 in range(0, NV, 8):
                            for j in range(NT):
                                ks[i] = after(ks[i], s[r0:r0 + 8, j * LANES:(j + 1) * LANES])
                    if c + 1 < NC:
                        lookahead.append(vpu_scores(odd, qb, c + 1, on_partial))
                    else:
                        lookahead.append(vpu_scores(ahead[1], ahead[2], 0, on_partial))

                def values():
                    p = jnp.concatenate([jnp.concatenate(
                        [pltpu.bitcast(p_u[zz["p"], cur, c, i, j], BF16) for j in range(NT)], axis=1)
                        for i in range((CH - NV) // 16)] + [p_vpu], axis=0)
                    o = _dot(v_s[pair, c, odd * HROWS:(odd + 1) * HROWS, :], p)
                    return o if c == 0 else o + acc

                pv_first = cfg["flip"] and qb * NC + c >= NQB * NC - cfg["flip"]
                if pv_first:
                    acc = values()
                s = mxu_scores(ahead[0], q, nxt, c, on_keys)
                if not pv_first:
                    acc = values()
                p_vpu = lookahead[0]
                store_p(nxt, c, s)
                anchor = s[0:8, 0:LANES]
                t = qb * NC + c
                if not cfg.get('nokb'): make_kb(next_pair, 1 - odd, t // NQB, (t % NQB) * DH // NQB, (t % NQB + 1) * DH // NQB, anchor)
                nmk = cfg["nmk"]
                cq = c - cfg["qstart"]
                if 0 <= cq < nmk and not cfg.get('noqb'):
                    d0, d1 = cq * DH // nmk, (cq + 1) * DH // nmk
                    if qb > 0:
                        make_qb(next_pair, 1 - odd, qb - 1, d0, d1, anchor)
                    else:
                        make_qb(pair, odd, NQB - 1, d0, d1, anchor)
            store_out(pair, odd, qb, acc)
            sums = acc[0:8] if odd else acc[16:24]
            sum_lo, sum_hi = jnp.minimum(sum_lo, sums), jnp.maximum(sum_hi, sums)
        pv_s[...] = p_vpu
        range_s[odd, 0], range_s[odd, 1] = sum_lo, sum_hi

    def head_step(h, _):
        for odd in range(2):
            pl.when(h % 2 == odd)(functools.partial(head_body, h // 2, odd))
        return 0

    if cfg.get("merged"):
        def pair_step(pair, _):
            head_body(pair, 0)
            head_body(pair, 1)
            return 0
        lax.fori_loop(0, cfg.get('nh', H) // 2, pair_step, 0)
    else:
        lax.fori_loop(0, cfg.get('nh', H), head_step, 0)

    sum_lo = jnp.where(qrow >= 4, range_s[0, 0], range_s[1, 0])
    sum_hi = jnp.where(qrow >= 4, range_s[0, 1], range_s[1, 1])
    safe = (sum_lo >= SUM_LO) & (sum_hi <= SUM_HI)
    unsafe = jnp.maximum(jnp.max(jnp.where(safe, 0.0, 1.0)), jnp.max(jnp.where(vmax_s[...] <= VALUE_HI, 0.0, 1.0)))

    @pl.when(unsafe > (0.0 if 'nh' not in cfg else 5.0))
    def _():
        def item(i, _):
            pair, qb = i // NQB, i % NQB
            k = pltpu.bitcast(k_s[pair], BF16)
            for odd in range(2):
                q = q_weights(pair, odd, qb)
                s = _dot(k[:, :q.shape[0]], q)
                p = jnp.exp2(s - jnp.max(s, axis=0, keepdims=True)).astype(BF16)
                store_out(pair, odd, qb, _dot(jnp.concatenate([v_s[pair, c, odd * HROWS:(odd + 1) * HROWS, :] for c in range(NC)], axis=1), p))
            return 0

        lax.fori_loop(0, NPAIR * NQB, item, 0)

    for c in cp_late:
        c.wait()
    b1 = b1_s[...].astype(F32).reshape(1, -1)
    b2 = b2_s[...].astype(F32).reshape(1, -1)
    n_fb = S // FB

    def attn_out(r):
        rows = rows_of(r, FB)
        row = lax.broadcasted_iota(jnp.int32, (8, FB), 0)
        ot = []
        for pair in range(NPAIR):
            acc = o_s[pair, :, rows]
            inv_even, inv_odd = 1.0 / acc[DH:DH + 1], 1.0 / acc[HROWS:HROWS + 1]
            ot += [acc[0:16] * inv_even, jnp.where(row < 4, acc[16:24] * inv_even, acc[24:32] * inv_odd),
                   acc[32:48] * inv_odd]
        hid = x_s[rows, :].astype(F32) + _dot(jnp.concatenate(ot, axis=0).T.astype(BF16), wo_s[...])
        h_s[rows, :] = hid
        ln_s[rows, :] = _layernorm(hid).astype(BF16)

    def ffn_up(r):
        a = jnp.maximum(_dot(ln_s[rows_of(r, FB), :], w1_s[...]) + b1, 0.0)
        return (a * a).astype(BF16)

    def ffn_down(r, a):
        rows = rows_of(r, FB)
        out_s[rows, :] = (h_s[rows, :] + (_dot(a, w2_s[...]) + b2)).astype(out_s.dtype)

    def write_back(r):
        rows = rows_of(r, FB)
        return pltpu.make_async_copy(out_s.at[rows, :], out_hbm.at[0, rows, :], out_sem.at[r])

    if cfg.get("only2") or cfg.get("stop") == 3:
        return
    attn_out(0)
    def p3_step(r):
        a = ffn_up(r)
        attn_out(r + 1)
        ffn_down(r, a)
        write_back(r).start()

    if cfg["loop3"]:
        u = cfg["loop3"]
        n_it = (n_fb - 1) // u

        def p3_body(i, _):
            for j in range(u):
                p3_step(i * u + j)
            return 0

        lax.fori_loop(0, n_it, p3_body, 0)
        for r in range(n_it * u, n_fb - 1):
            p3_step(r)
    else:
        for r in range(n_fb - 1):
            p3_step(r)
    ffn_down(n_fb - 1, ffn_up(n_fb - 1))
    if not cfg.get("nowb"):
        write_back(n_fb - 1).start()
    for r in range(n_fb - cfg.get("nowb", 0)):
        write_back(r).wait()


def build(cfg):
    def fn(A_x, A_wqkv, A_wo, B_x, B_w1, B_b1, B_w2, B_b2):
        del B_x
        _, S, D = A_x.shape
        H = NUM_HEADS
        hbm = pl.BlockSpec(memory_space=pl.ANY)
        scratch = [
            pltpu.VMEM((S, D), A_x.dtype),
            pltpu.VMEM((D, D), A_wqkv.dtype),
            pltpu.VMEM((D, D), A_wqkv.dtype),
            pltpu.VMEM((D, D), A_wqkv.dtype),
            pltpu.VMEM(A_wo.shape, A_wo.dtype),
            pltpu.VMEM(B_w1.shape, B_w1.dtype),
            pltpu.VMEM(B_b1.shape, B_b1.dtype),
            pltpu.VMEM(B_w2.shape, B_w2.dtype),
            pltpu.VMEM(B_b2.shape, B_b2.dtype),
            pltpu.VMEM((S, D), BF16),
            pltpu.VMEM((S, D), F32),
            pltpu.VMEM((H // 2, S // 2, LANES), U32),
            pltpu.VMEM((D, S), F32),
            pltpu.VMEM((H // 2, S // CH, 2 * HROWS, CH), F32),
            pltpu.VMEM((1, 2, S // CH, (CH - NV) // 16, NQ // LANES, 16, LANES) if cfg["play"] else (2, NQ // LANES, S // CH * (CH - NV), LANES), BF16),
            pltpu.VMEM((1, 2, S // CH, D // H, NV, LANES), F32),
            pltpu.VMEM((1, S // NQ, D // H, 8, NQ), F32),
            pltpu.VMEM((NV, NQ), BF16),
            pltpu.VMEM((2, 2, 8, NQ), F32),
            pltpu.VMEM((8, LANES), F32),
            pltpu.VMEM((H // 2, 2 * HROWS, S), F32),
            pltpu.VMEM((S, D), A_x.dtype),
            pltpu.SMEM((1,), jnp.int32),
            pltpu.SemaphoreType.DMA((11,)),
            pltpu.SemaphoreType.DMA((S // cfg["FB"],)),
        ]
        return pl.pallas_call(
            functools.partial(_kernel, cfg=cfg),
            out_shape=jax.ShapeDtypeStruct(A_x.shape, A_x.dtype),
            in_specs=[hbm] * 7,
            out_specs=hbm,
            scratch_shapes=scratch,
            compiler_params=pltpu.CompilerParams(vmem_limit_bytes=110 * 2**20, flags=cfg.get("flags")),
        )(A_x, A_wqkv, A_wo, B_w1, B_b1, B_w2, B_b2)
    return fn


@jax.jit
def pallas_sequential_preLN__softmax_full_mha__dense_activation_squared_relu__prompt_kernel(
    A_x: jax.Array,
    A_wqkv: jax.Array,
    A_wo: jax.Array,
    B_x: jax.Array,
    B_w1: jax.Array,
    B_b1: jax.Array,
    B_w2: jax.Array,
    B_b2: jax.Array,
):
    return build(CFG)(A_x, A_wqkv, A_wo, B_x, B_w1, B_b1, B_w2, B_b2)
```

```python
import functools
import math

import jax
import jax.numpy as jnp
from jax import lax
import jax.experimental.pallas as pl
import jax.experimental.pallas.tpu as pltpu

BF16 = jnp.bfloat16
F32 = jnp.float32
U32 = jnp.uint32

NUM_HEADS = 32
LN_EPS = 1e-5
LANES = 128
NQ = 512
CH = 128
NV = 16
HROWS = 24
FAST = 512
SUM_LO, SUM_HI = 2.0 ** -20, 2.0 ** 90
VALUE_HI = 2.0 ** 36
RB = 512
PB = 256
FB = 256
QV_ORDER, WO_ORDER, UP_ORDER, DOWN_ORDER = "12x43056", "xy4302615", "12x43056", "3x024516"
KEY_MARKS = (2, 3, 4, 5, 6)


def _dot(a, b):
    return jnp.dot(a, b, preferred_element_type=F32)


def _layernorm(x):
    mean = jnp.mean(x, axis=-1, keepdims=True)
    xc = x - mean
    var = jnp.mean(xc * xc, axis=-1, keepdims=True)
    return xc * lax.rsqrt(var + LN_EPS)


def _quadrants(a):
    m, n = a.shape[0] // 2, a.shape[1] // 2
    return a[:m, :n], a[:m, n:], a[m:, :n], a[m:, n:]


def _strassen_lhs(a):
    a11, a12, a21, a22 = _quadrants(a)
    return a11 + a22, a21 + a22, a11, a22, a11 + a12, a21 - a11, a12 - a22


def _strassen_rhs(b11, b12, b21, b22):
    return b11 + b22, b11, b12 - b22, b21 - b11, b22, b11 + b12, b21 + b22


def _strassen_matmul(lhs, rhs_ref, order, others):
    words = rhs_ref.bitcast(U32)
    m, results = {}, {}
    for c in order:
        if c.isdigit():
            i = int(c)
            rhs = jnp.concatenate(
                [jnp.concatenate([pltpu.bitcast(words[i, r, j], BF16) for j in range(rhs_ref.shape[2])], axis=1)
                 for r in range(rhs_ref.shape[1])], axis=0)
            m[i] = _dot(lhs(i), rhs)
        elif c in others:
            results[c] = others[c]()

    top = jnp.concatenate([m[0] + m[3] - m[4] + m[6], m[2] + m[4]], axis=1)
    bottom = jnp.concatenate([m[1] + m[3], m[0] - m[1] + m[2] + m[5]], axis=1)
    return jnp.concatenate([top, bottom], axis=0), results, [m[int(c)] for c in order if c.isdigit()]


def _share(jobs, i, n):
    return jobs[i * len(jobs) // n:(i + 1) * len(jobs) // n]


def _kernel(x_hbm, wqkv_hbm, wo_hbm, w1_hbm, b1_hbm, w2_hbm, b2_hbm, out_hbm,
            x_s, wq_s, wk_s, wv_s, wo_s, w1_s, b1_s, w2_s, b2_s,
            wqv_x, wo_x, w1_x, w2_x, ln_s, lnx_s, h_s, out_s,
            k_s, q_s, v_s, p_s, kb_s, qb_s, pv_s, o_s, range_s, vmax_s, never_s, zero_s,
            in_sem, out_sem):
    S, D = x_s.shape
    DH = D // NUM_HEADS
    NPAIR = NUM_HEADS // 2
    NT, NC, NQB = NQ // LANES, S // CH, S // NQ
    KA = 3 * LANES
    q_scale = DH ** -0.5 * math.log2(math.e)

    def rows_of(r, n):
        return pl.ds(r * n, n) if isinstance(r, int) else pl.ds(pl.multiple_of(r * n, n), n)

    def fetch(i, src, dst):
        return pltpu.make_async_copy(src, dst, in_sem.at[i])

    cp_x0 = fetch(0, x_hbm.at[0, pl.ds(0, RB), :], x_s.at[pl.ds(0, RB), :])
    cp_x1 = fetch(1, x_hbm.at[0, pl.ds(RB, RB), :], x_s.at[pl.ds(RB, RB), :])
    cp_x2 = fetch(2, x_hbm.at[0, pl.ds(2 * RB, S - 2 * RB), :], x_s.at[pl.ds(2 * RB, S - 2 * RB), :])
    cp_wka = fetch(3, wqkv_hbm.at[:, pl.ds(D, KA)], wk_s.at[:, pl.ds(0, KA)])
    cp_wkb = fetch(4, wqkv_hbm.at[:, pl.ds(D + KA, D - KA)], wk_s.at[:, pl.ds(KA, D - KA)])
    cp_wq = fetch(5, wqkv_hbm.at[:, pl.ds(0, D)], wq_s)
    cp_wv = fetch(6, wqkv_hbm.at[:, pl.ds(2 * D, D)], wv_s)
    cp_b2 = fetch(7, b2_hbm, b2_s)
    cp_late = [fetch(8, wo_hbm, wo_s), fetch(9, w1_hbm, w1_s), fetch(10, b1_hbm, b1_s), fetch(11, w2_hbm, w2_s)]
    cp_x0.start()
    cp_b2.start()
    cp_wka.start()
    cp_wkb.start()

    vmax_s[...] = jnp.zeros(vmax_s.shape, F32)
    never_s[...] = jnp.zeros(never_s.shape, jnp.int32)
    zero_s[0] = 0

    def after(x, y):
        if x.dtype != y.dtype:
            y = pltpu.bitcast(y, x.dtype)
        return jnp.where(never_s[...] != 0, y, x)

    def first_tile_after(x, anchor):
        head = jnp.concatenate([after(x[0:8, 0:LANES], anchor), after(x[8:16, 0:LANES], anchor)], axis=0)
        return jnp.concatenate([head, x[:, LANES:]], axis=1)

    def run_jobs(jobs, results, row_step):
        anchors = [a[r:r + 8, c:c + LANES] for a in results
                   for r in range(0, a.shape[0], row_step) for c in range(0, a.shape[1], LANES)]
        for i, job in enumerate(jobs):
            job(anchors[i * len(anchors) // len(jobs)])

    def norm_job(lo):
        def run(anchor):
            ln_s[lo:lo + 16, :] = _layernorm(first_tile_after(x_s[lo:lo + 16, :].astype(F32), anchor)).astype(BF16)
        return run

    def weight_jobs(dst, weight):
        n_rows, n_tiles = dst.shape[1] * 16, dst.shape[2]

        def job(r, j):
            def run(anchor):
                b11, b12, b21, b22 = (weight(a * n_rows + r, (b * n_tiles + j) * LANES).astype(F32)
                                      for a in range(2) for b in range(2))
                b11, b22 = (jnp.concatenate([after(t[0:8], anchor), after(t[8:16], anchor)], axis=0)
                            for t in (b11, b22))
                for i, t in enumerate(_strassen_rhs(b11, b12, b21, b22)):
                    dst[i, r // 16, j] = t.astype(BF16)
            return run
        return [job(r, j) for r in range(0, n_rows, 16) for j in range(n_tiles)]

    def tile_of(ref):
        return lambda r, c: ref[r:r + 16, c:c + LANES]

    def normalize(lo, n):
        ln_s[lo:lo + n, :] = _layernorm(x_s[lo:lo + n, :].astype(F32)).astype(BF16)

    def project_k(lo, n, jobs=(), first=None):
        k = _dot(ln_s[lo:lo + n, :], wk_s[...] if first is None else wk_s[:, KA:])
        run_jobs(jobs, [k], 32)
        k = k.astype(BF16) if first is None else jnp.concatenate([first, k.astype(BF16)], axis=1)
        slabs = [pltpu.bitcast(k[:, j:j + LANES], U32) for j in range(0, D, LANES)]
        lane = lax.broadcasted_iota(jnp.int32, (n // 2, LANES), 1)
        for pair in range(NPAIR):
            j, off = divmod(pair * 2 * DH, LANES)
            kp = slabs[j]
            if off + 2 * DH > LANES:
                kp = jnp.where(lane >= LANES // 2, kp, slabs[j + 1])
            if off:
                kp = pltpu.roll(kp, LANES - off, 1)
            k_s[pair, lo // 2:(lo + n) // 2, :] = kp

    def project_qv(lo, n, fast, jobs=()):
        if fast:
            lhs = _strassen_lhs(ln_s[lo:lo + n, :FAST].astype(F32))

            def tail():
                ln = ln_s[lo:lo + n, FAST:]
                return _dot(ln, wq_s[FAST:, :]), _dot(ln, wv_s[FAST:, :])
            qv, rest, products = _strassen_matmul(lambda i: lhs[i].astype(BF16), wqv_x, QV_ORDER, dict(x=tail))
            q, v = qv[:, :D] + rest["x"][0], qv[:, D:] + rest["x"][1]
            run_jobs(jobs, products, 64)
        else:
            ln = ln_s[lo:lo + n, :]
            q, v = _dot(ln, wq_s[...]), _dot(ln, wv_s[...])
            run_jobs(jobs, [q, v], 32)
        q_s[:, lo:lo + n] = (q * q_scale).T
        vt = v.astype(BF16).astype(F32).T
        vmax = jnp.max(jnp.abs(vt).reshape(D // 8, 8, n), axis=0)
        row = lax.broadcasted_iota(jnp.int32, (8, n), 0)
        for j in range(n // CH):
            vmax_s[...] = jnp.maximum(vmax_s[...], vmax[:, j * CH:(j + 1) * CH])
        for pair in range(NPAIR):
            top = pair * 2 * DH
            mid = vt[top + 16:top + 24]
            both = jnp.concatenate([vt[top:top + 16], jnp.where(row < 4, mid, 1.0),
                                    jnp.where(row >= 4, mid, 1.0), vt[top + 24:top + 40]], axis=0)
            for j in range(n // CH):
                v_s[pair, lo // CH + j] = both[:, j * CH:(j + 1) * CH]

    cp_x0.wait()
    normalize(0, RB)
    cp_wka.wait()
    cp_x1.start()
    cp_wq.start()
    cp_wv.start()
    cp_b2.wait()
    firsts = [_dot(ln_s[lo:lo + LANES, :], wk_s[:, :KA]).astype(BF16) for lo in range(0, RB, LANES)]
    cp_wkb.wait()
    cp_x2.start()
    cp_x1.wait()
    jobs = [norm_job(lo) for lo in range(RB, 2 * RB, 16)]
    for i, first in enumerate(firsts):
        project_k(i * LANES, LANES, _share(jobs, i, len(firsts)), first)
    for lo in range(RB, 2 * RB, LANES):
        project_k(lo, LANES)
    for cp in cp_late:
        cp.start()
    cp_wq.wait()
    cp_wv.wait()
    project_qv(0, PB, False, weight_jobs(wqv_x, lambda r, c: tile_of(wq_s if c < D else wv_s)(r, c % D)))
    cp_x2.wait()
    project_qv(PB, PB, True, [norm_job(lo) for lo in range(2 * RB, S, 16)])
    for lo in range(2 * RB, S, PB):
        project_k(lo, PB)
    for cp in cp_late:
        cp.wait()
    jobs = weight_jobs(w1_x, tile_of(w1_s)) + weight_jobs(w2_x, tile_of(w2_s))
    jobs += weight_jobs(wo_x, tile_of(wo_s))
    blocks = range(2 * PB, S, PB)
    for i, lo in enumerate(blocks):
        project_qv(lo, PB, True, _share(jobs, i, len(blocks)))

    p_words = p_s.bitcast(U32)
    qrow = lax.broadcasted_iota(jnp.int32, (8, NQ), 0)

    def q_rows(pair, lo, n):
        start = pair * 2 * DH + lo
        return pl.ds(start if isinstance(start, int) else pl.multiple_of(start, 8), n)

    def head_rows(odd):
        return pl.ds(odd * HROWS, HROWS)

    def q_weights(pair, odd, qb):
        cols = rows_of(qb, NQ)
        mid = q_s[q_rows(pair, 16, 8), cols]
        zero = jnp.zeros((8, NQ), F32)
        if odd:
            parts = [zero, zero, jnp.where(qrow >= 4, mid, 0.0), q_s[q_rows(pair, 24, 16), cols], zero]
        else:
            parts = [q_s[q_rows(pair, 0, 16), cols], jnp.where(qrow < 4, mid, 0.0), zero]
        return jnp.concatenate(parts, axis=0).astype(BF16)

    def spread_k(z, pair, odd, c, dims, anchor=None):
        k = k_s[pair, ((c + 1) * CH - NV) // 2:(c + 1) * CH // 2, :]
        if anchor is not None:
            k = after(k, anchor)
        k = pltpu.bitcast(k, BF16).astype(F32)
        for d in dims:
            kb_s[z, odd, c, d] = jnp.broadcast_to(k[:, odd * DH + d:odd * DH + d + 1], (NV, LANES))

    def spread_q(z, pair, odd, qb, dims, anchor=None):
        for d in dims:
            r = odd * DH + d
            q = q_s[q_rows(pair, r // 8 * 8, 8), rows_of(qb, NQ)]
            if anchor is not None:
                q = jnp.concatenate([after(q[:, j:j + LANES], anchor) for j in range(0, NQ, LANES)], axis=1)
            qb_s[z, qb, d] = jnp.broadcast_to(q[r % 8:r % 8 + 1, :], (8, NQ))

    def vector_probs(z, odd, qb, c, keys=None):
        s = None
        for piece in range(len(KEY_MARKS) + 1):
            for d in _share(range(DH), piece, len(KEY_MARKS) + 1):
                t = (jnp.concatenate([kb_s[z, odd, c, d]] * NT, axis=1)
                     * jnp.concatenate([qb_s[z, qb, d]] * (NV // 8), axis=0))
                s = t if s is None else s + t
            if keys is not None and piece < len(KEY_MARKS):
                for r in range(0, NV, 8):
                    for j in range(0, NQ, LANES):
                        keys[KEY_MARKS[piece]] = after(keys[KEY_MARKS[piece]], s[r:r + 8, j:j + LANES])
        return jnp.exp2(s).astype(BF16)

    def key_tiles(pair, c):
        return [k_s[pair, (c * CH + i) // 2:(c * CH + i) // 2 + 8, :] for i in range(0, CH - NV, 16)]

    def mxu_scores(keys, q):
        k = pltpu.bitcast(jnp.concatenate(keys, axis=0), BF16)
        return _dot(k[:, :q.shape[0]], q)

    def store_probs(z, slot, c, s):
        p = jnp.exp2(s)
        for i in range((CH - NV) // 16):
            for j in range(NT):
                p_s[z, slot, c, i, j] = p[16 * i:16 * (i + 1), j * LANES:(j + 1) * LANES].astype(BF16)

    def attention_rows(r):
        row = lax.broadcasted_iota(jnp.int32, (8, FB), 0)
        parts = []
        for pair in range(NPAIR):
            acc = o_s[pair, :, rows_of(r, FB)]
            inv_even, inv_odd = 1.0 / acc[DH:DH + 1], 1.0 / acc[HROWS:HROWS + 1]
            parts += [acc[0:16] * inv_even, jnp.where(row < 4, acc[16:24] * inv_even, acc[24:32] * inv_odd),
                      acc[32:48] * inv_odd]
        return jnp.concatenate(parts, axis=0).T

    def residual_norm(r, proj):
        rows = rows_of(r, FB)
        hid = x_s[rows, :].astype(F32) + proj
        h_s[rows, :] = hid
        ln = _layernorm(hid)
        ln_s[rows, FAST:] = ln[:, FAST:].astype(BF16)
        for i, a in enumerate(_strassen_lhs(ln[:, :FAST])):
            lnx_s[r % 2, i] = a.astype(BF16)

    for c in range(NC):
        spread_k(0, 0, 0, c, range(DH))
    for qb in range(NQB):
        spread_q(0, 0, 0, qb, range(DH))
    q_first = q_weights(0, 0, 0)
    for c in range(NC):
        store_probs(0, 0, c, mxu_scores(key_tiles(0, c), q_first))
    pv_s[...] = vector_probs(0, 0, 0, 0)
    range_s[...] = jnp.ones(range_s.shape, F32)

    def head(pair, odd, final=False):
        p_vec, sum_lo, sum_hi = pv_s[...], range_s[odd, 0], range_s[odd, 1]
        z = zero_s[0]
        for qb in range(NQB):
            ahead = (pair, odd, qb + 1) if qb + 1 < NQB else (pair + odd, 1 - odd, 0)
            drain = final and qb + 1 == NQB
            if drain:
                o_first = attention_rows(0).astype(BF16)
            else:
                q = q_weights(*ahead)
            for c in range(NC):
                keys = None if drain else key_tiles(ahead[0], c)
                if c + 1 < NC:
                    p_next = vector_probs(z, odd, qb, c + 1, keys)
                elif not drain:
                    p_next = vector_probs(z, ahead[1], ahead[2], 0, keys)
                if not drain:
                    s = mxu_scores(keys, q)
                elif 0 <= c - 3 < D // LANES:
                    j = (c - 3) * LANES
                    part = _dot(o_first[:, j:j + LANES], wo_s[j:j + LANES, :])
                    proj = part if j == 0 else part + proj
                    if j + LANES == D:
                        residual_norm(0, proj)
                p = jnp.concatenate(
                    [jnp.concatenate([pltpu.bitcast(p_words[z, qb % 2, c, i, j], BF16) for j in range(NT)], axis=1)
                     for i in range((CH - NV) // 16)] + [p_vec], axis=0)
                o = _dot(v_s[pair, c, head_rows(odd), :], p)
                acc = o if c == 0 else o + acc
                p_vec = p_next
                if drain:
                    continue
                store_probs(z, (qb + 1) % 2, c, s)
                anchor = s[0:8, 0:LANES]
                group, part_of = divmod(qb * NC + c, NQB)
                if not final:
                    spread_k(z, pair + odd, 1 - odd, group, _share(range(DH), part_of, NQB), anchor)
                if 0 <= c - 3 < DH // 2:
                    dims = _share(range(DH), c - 3, DH // 2)
                    if qb == 0:
                        spread_q(z, pair, odd, NQB - 1, dims, anchor)
                    elif not final:
                        spread_q(z, pair + odd, 1 - odd, qb - 1, dims, anchor)
            o_s[pair, head_rows(odd), rows_of(qb, NQ)] = acc
            sums = acc[0:8] if odd else acc[16:24]
            sum_lo, sum_hi = jnp.minimum(sum_lo, sums), jnp.maximum(sum_hi, sums)
        pv_s[...] = p_vec
        range_s[odd, 0], range_s[odd, 1] = sum_lo, sum_hi

    def head_step(h, _):
        for odd in range(2):
            pl.when(h % 2 == odd)(functools.partial(head, h // 2, odd))
        return 0

    lax.fori_loop(0, NUM_HEADS - 1, head_step, 0)
    head(NPAIR - 1, 1, final=True)

    sum_lo = jnp.where(qrow >= 4, range_s[0, 0], range_s[1, 0])
    sum_hi = jnp.where(qrow >= 4, range_s[0, 1], range_s[1, 1])
    unsafe = jnp.maximum(jnp.max(jnp.where((sum_lo >= SUM_LO) & (sum_hi <= SUM_HI), 0.0, 1.0)),
                         jnp.max(jnp.where(vmax_s[...] <= VALUE_HI, 0.0, 1.0)))

    @pl.when(unsafe > 0.0)
    def _():
        def exact(i, _):
            pair, qb = i // NQB, i % NQB
            k = pltpu.bitcast(k_s[pair], BF16)
            for odd in range(2):
                q = q_weights(pair, odd, qb)
                s = _dot(k[:, :q.shape[0]], q)
                p = jnp.exp2(s - jnp.max(s, axis=0, keepdims=True)).astype(BF16)
                v = jnp.concatenate([v_s[pair, c, head_rows(odd), :] for c in range(NC)], axis=1)
                o_s[pair, head_rows(odd), rows_of(qb, NQ)] = _dot(v, p)
            return 0

        lax.fori_loop(0, NPAIR * NQB, exact, 0)
        residual_norm(0, _dot(attention_rows(0).astype(BF16), wo_s[...]))

    b1 = b1_s[...].astype(F32).reshape(1, -1)
    b2 = b2_s[...].astype(F32).reshape(1, -1)

    def project_out(r):
        o = attention_rows(r)
        lhs = _strassen_lhs(o[:, :FAST])
        fast, rest, _ = _strassen_matmul(lambda i: lhs[i].astype(BF16), wo_x, WO_ORDER, dict(
            x=lambda: _dot(o[:, FAST:].astype(BF16), wo_s[FAST:, :]),
            y=lambda: _dot(o[:, :FAST].astype(BF16), wo_s[:FAST, FAST:])))
        residual_norm(r, jnp.concatenate([fast, rest["y"]], axis=1) + rest["x"])

    def ffn(r, meanwhile=lambda: None):
        rows = rows_of(r, FB)
        lhs = [lnx_s[r % 2, i] for i in range(7)]
        ln_rest = ln_s[rows, FAST:]
        fast, rest, _ = _strassen_matmul(lambda i: lhs[i], w1_x, UP_ORDER, dict(
            x=lambda: _dot(ln_rest, w1_s[FAST:, :])))
        meanwhile()
        act = jnp.square(jnp.maximum(fast + rest["x"] + b1, 0.0))
        lhs = _strassen_lhs(act)
        fast, rest, _ = _strassen_matmul(lambda i: lhs[i].astype(BF16), w2_x, DOWN_ORDER, dict(
            x=lambda: _dot(act.astype(BF16), w2_s[:, FAST:])))
        y = jnp.concatenate([fast, rest["x"]], axis=1)
        out_s[rows, :] = (h_s[rows, :] + (y + b2)).astype(out_s.dtype)

    def write_back(r):
        return pltpu.make_async_copy(out_s.at[rows_of(r, FB), :], out_hbm.at[0, rows_of(r, FB), :], out_sem.at[r])

    def block_step(r, _):
        ffn(r, lambda: project_out(r + 1))
        write_back(r).start()
        return 0

    n_blocks = S // FB
    lax.fori_loop(0, n_blocks - 1, block_step, 0)
    ffn(n_blocks - 1)
    write_back(n_blocks - 1).start()
    for r in range(n_blocks):
        write_back(r).wait()


@jax.jit
def pallas_sequential_preLN__softmax_full_mha__dense_activation_squared_relu__prompt_kernel(
    A_x: jax.Array,
    A_wqkv: jax.Array,
    A_wo: jax.Array,
    B_x: jax.Array,
    B_w1: jax.Array,
    B_b1: jax.Array,
    B_w2: jax.Array,
    B_b2: jax.Array,
):
    del B_x
    _, S, D = A_x.shape
    F = B_w1.shape[1]
    pairs, dh = NUM_HEADS // 2, D // NUM_HEADS
    vmem = pltpu.VMEM
    scratch = [
        vmem((S, D), A_x.dtype),
        vmem((D, D), A_wqkv.dtype), vmem((D, D), A_wqkv.dtype), vmem((D, D), A_wqkv.dtype),
        vmem(A_wo.shape, A_wo.dtype),
        vmem(B_w1.shape, B_w1.dtype), vmem(B_b1.shape, B_b1.dtype),
        vmem(B_w2.shape, B_w2.dtype), vmem(B_b2.shape, B_b2.dtype),
        vmem((7, FAST // 32, D // LANES, 16, LANES), BF16),
        vmem((7, FAST // 32, FAST // 2 // LANES, 16, LANES), BF16),
        vmem((7, FAST // 32, F // 2 // LANES, 16, LANES), BF16),
        vmem((7, F // 32, FAST // 2 // LANES, 16, LANES), BF16),
        vmem((S, D), BF16),
        vmem((2, 7, FB // 2, FAST // 2), BF16),
        vmem((S, D), F32),
        vmem((S, D), A_x.dtype),
        vmem((pairs, S // 2, LANES), U32),
        vmem((D, S), F32),
        vmem((pairs, S // CH, 2 * HROWS, CH), F32),
        vmem((1, 2, S // CH, (CH - NV) // 16, NQ // LANES, 16, LANES), BF16),
        vmem((1, 2, S // CH, dh, NV, LANES), F32),
        vmem((1, S // NQ, dh, 8, NQ), F32),
        vmem((NV, NQ), BF16),
        vmem((pairs, 2 * HROWS, S), F32),
        vmem((2, 2, 8, NQ), F32),
        vmem((8, CH), F32),
        vmem((8, LANES), jnp.int32),
        pltpu.SMEM((1,), jnp.int32),
        pltpu.SemaphoreType.DMA((12,)),
        pltpu.SemaphoreType.DMA((S // FB,)),
    ]
    hbm = pl.BlockSpec(memory_space=pl.ANY)
    return pl.pallas_call(
        _kernel,
        out_shape=jax.ShapeDtypeStruct(A_x.shape, A_x.dtype),
        in_specs=[hbm] * 7,
        out_specs=hbm,
        scratch_shapes=scratch,
        compiler_params=pltpu.CompilerParams(vmem_limit_bytes=100 * 2 ** 20),
    )(A_x, A_wqkv, A_wo, B_w1, B_b1, B_w2, B_b2)
```

```python
import functools
import math

import numpy as np

import jax
import jax.numpy as jnp
from jax import lax
import jax.experimental.pallas as pl
import jax.experimental.pallas.tpu as pltpu

BF16 = jnp.bfloat16
F32 = jnp.float32
U32 = jnp.uint32

NUM_HEADS = 32
LN_EPS = 1e-5
LANES = 128
NQ = 512
CH = 128
NV = 16
HROWS = 24
FAST = 512
SUM_LO, SUM_HI = 2.0 ** -20, 2.0 ** 90
VALUE_HI = 2.0 ** 36
RB = 512
PB = 256
FB = 256
QKV_ORDER, WO_ORDER = "2y4x13065", "4y0362x15"
FFN_ORDER = "fbgtvmoncwjrykpisqxahdelu", "biwmgntlejfosqhrxyvkpdcua"
LAST_FFN_ORDER = "fkbjytglporwsqmncvxahdieu", "blimgqhoprtyjfxwsvunedcka"
PROJECT_AT = 31
KEY_MARKS = (2, 3, 4, 5, 6)


def _dot(a, b):
    return jnp.dot(a, b, preferred_element_type=F32)


def _layernorm(x):
    mean = jnp.mean(x, axis=-1, keepdims=True)
    xc = x - mean
    var = jnp.mean(xc * xc, axis=-1, keepdims=True)
    return xc * lax.rsqrt(var + LN_EPS)


def _quadrants(a):
    m, n = a.shape[0] // 2, a.shape[1] // 2
    return a[:m, :n], a[:m, n:], a[m:, :n], a[m:, n:]


def _strassen_lhs(a):
    a11, a12, a21, a22 = _quadrants(a)
    return a11 + a22, a21 + a22, a11, a22, a11 + a12, a21 - a11, a12 - a22


def _strassen_rhs(b11, b12, b21, b22):
    return b11 + b22, b11, b12 - b22, b21 - b11, b22, b11 + b12, b21 + b22


def _strassen_matmul(lhs, rhs_ref, order, others):
    words = rhs_ref.bitcast(U32)
    m, results = {}, {}
    for c in order:
        if c.isdigit():
            i = int(c)
            rhs = jnp.concatenate(
                [jnp.concatenate([pltpu.bitcast(words[i, r, j], BF16) for j in range(rhs_ref.shape[2])], axis=1)
                 for r in range(rhs_ref.shape[1])], axis=0)
            m[i] = _dot(lhs(i), rhs)
        elif c in others:
            results[c] = others[c]()

    top = jnp.concatenate([m[0] + m[3] - m[4] + m[6], m[2] + m[4]], axis=1)
    bottom = jnp.concatenate([m[1] + m[3], m[0] - m[1] + m[2] + m[5]], axis=1)
    return jnp.concatenate([top, bottom], axis=0), results, [m[int(c)] for c in order if c.isdigit()]


_SCHEME = (
    ("-.........", "++-....-+......", "..+..."),
    ("-.-..+.+..", ".+.............", "....+."),
    ("...+-.....", "...........+...", "+.++.+"),
    (".+......-.", "....-....-.+...", ".-.+.."),
    ("...-....+.", ".........+-..-+", ".+...."),
    ("......+.-.", "....+..........", "...++."),
    ("-.-.......", ".......-+......", ".+..+."),
    ("..+.-..-..", "......-.....-.+", ".--+.."),
    (".....+....", "..+..+.........", ".....+"),
    ("...-+...+.", "...........+.-+", ".-.+.+"),
    ("..+.-.....", "......+........", "+..+.."),
    ("..-.+..+.-", "............-.+", "...+.."),
    (".........+", ".............+.", "...+++"),
    (".......+..", "........+......", ".++.++"),
    ("...+-...-+", ".............-+", "...+.+"),
    ("..+....-..", ".-....-+....-.+", ".++..."),
    (".-........", "...-.+...-.+...", "+..+.."),
    ("....+.....", "......+....++..", "+++..."),
    (".....-+...", ".....+.........", "+.++.+"),
    ("+.+....-..", ".+.....-+......", ".++.+."),
    (".+....-...", "-..-+..........", "...+.."),
    (".+...+-...", "+....+.........", "+.++.."),
    ("........+.", "....+.....+....", ".+..+."),
    (".+.-......", ".........-.+...", "++...."),
    ("+-...-+...", "+..............", "+.+..."),
)
_SIGN = {"+": 1, "-": -1, ".": 0}
_A, _B, _C = (np.array([[_SIGN[c] for c in row[i]] for row in _SCHEME]).reshape(-1, *shape)
              for i, shape in enumerate(((2, 5), (5, 3), (2, 3))))
WIDE_K = (_A, _B, _C)
WIDE_N = (_C, _B.transpose(0, 2, 1), _A)


def _blocks(x, rows, cols):
    m, n = x.shape[0] // rows, x.shape[1] // cols
    return [x[i * m:(i + 1) * m, j * n:(j + 1) * n] for i in range(rows) for j in range(cols)]


def _signed_sum(signs, terms):
    picked = sorted(((s, i) for i, s in enumerate(signs) if s), key=lambda e: -e[0])
    total = terms[picked[0][1]] if picked[0][0] > 0 else -terms[picked[0][1]]
    for s, i in picked[1:]:
        total = total + terms[i] if s > 0 else total - terms[i]
    return total


def _operands(signs, x):
    blocks = _blocks(x, *signs.shape[1:])
    return [_signed_sum(s.ravel(), blocks) for s in signs]


def _fast_matmul(scheme, lhs, rhs_ref, order, meanwhile=()):
    words = rhs_ref.bitcast(U32)
    products = [None] * len(order)
    for n, t in enumerate(order):
        for position, fn in meanwhile:
            if position == n:
                fn()
        rhs = jnp.concatenate(
            [jnp.concatenate([pltpu.bitcast(words[t, r, j], BF16) for j in range(rhs_ref.shape[2])], axis=1)
             for r in range(rhs_ref.shape[1])], axis=0)
        products[t] = _dot(lhs(t), rhs)
    signs = scheme[2]
    out = []
    for i in range(signs.shape[1]):
        row = []
        for k in range(signs.shape[2]):
            total = None
            for t in reversed(order):
                s = signs[t, i, k]
                if s and total is None:
                    total = products[t] if s > 0 else -products[t]
                elif s:
                    total = total + products[t] if s > 0 else total - products[t]
            row.append(total)
        out.append(jnp.concatenate(row, axis=1))
    return jnp.concatenate(out, axis=0)


def _share(jobs, i, n):
    return jobs[i * len(jobs) // n:(i + 1) * len(jobs) // n]


def _kernel(x_hbm, wqkv_hbm, wo_hbm, w1_hbm, b1_hbm, w2_hbm, b2_hbm, out_hbm,
            x_s, wq_s, wk_s, wv_s, wo_s, w1_s, b1_s, w2_s, b2_s,
            wq_x, wk_x, wv_x, wo_x, w1_x, w2_x, ln_s, lnx_s, h_s, out_s,
            k_s, q_s, v_s, p_s, kb_s, qb_s, pv_s, o_s, range_s, vmax_s, never_s, zero_s,
            in_sem, out_sem):
    S, D = x_s.shape
    DH = D // NUM_HEADS
    NPAIR = NUM_HEADS // 2
    NT, NC, NQB = NQ // LANES, S // CH, S // NQ
    KA = 3 * LANES
    q_scale = DH ** -0.5 * math.log2(math.e)

    def rows_of(r, n):
        return pl.ds(r * n, n) if isinstance(r, int) else pl.ds(pl.multiple_of(r * n, n), n)

    def fetch(i, src, dst):
        return pltpu.make_async_copy(src, dst, in_sem.at[i])

    cp_x0 = fetch(0, x_hbm.at[0, pl.ds(0, RB), :], x_s.at[pl.ds(0, RB), :])
    cp_x1 = fetch(1, x_hbm.at[0, pl.ds(RB, RB), :], x_s.at[pl.ds(RB, RB), :])
    cp_x2 = fetch(2, x_hbm.at[0, pl.ds(2 * RB, S - 2 * RB), :], x_s.at[pl.ds(2 * RB, S - 2 * RB), :])
    cp_wka = fetch(3, wqkv_hbm.at[:, pl.ds(D, KA)], wk_s.at[:, pl.ds(0, KA)])
    cp_wkb = fetch(4, wqkv_hbm.at[:, pl.ds(D + KA, D - KA)], wk_s.at[:, pl.ds(KA, D - KA)])
    cp_wq = fetch(5, wqkv_hbm.at[:, pl.ds(0, D)], wq_s)
    cp_wv = fetch(6, wqkv_hbm.at[:, pl.ds(2 * D, D)], wv_s)
    cp_b2 = fetch(7, b2_hbm, b2_s)
    cp_late = [fetch(8, wo_hbm, wo_s), fetch(9, w1_hbm, w1_s), fetch(10, b1_hbm, b1_s), fetch(11, w2_hbm, w2_s)]
    cp_x0.start()
    cp_b2.start()
    cp_wka.start()

    vmax_s[...] = jnp.zeros(vmax_s.shape, F32)
    never_s[...] = jnp.zeros(never_s.shape, jnp.int32)
    zero_s[0] = 0

    def after(x, y):
        if x.dtype != y.dtype:
            y = pltpu.bitcast(y, x.dtype)
        return jnp.where(never_s[...] != 0, y, x)

    def first_tile_after(x, anchor):
        head = jnp.concatenate([after(x[0:8, 0:LANES], anchor), after(x[8:16, 0:LANES], anchor)], axis=0)
        return jnp.concatenate([head, x[:, LANES:]], axis=1)

    def run_jobs(jobs, results, row_step):
        anchors = [a[r:r + 8, c:c + LANES] for a in results
                   for r in range(0, a.shape[0], row_step) for c in range(0, a.shape[1], LANES)]
        for i, job in enumerate(jobs):
            job(anchors[i * len(anchors) // len(jobs)])

    def norm_job(lo):
        def run(anchor):
            ln_s[lo:lo + 16, :] = _layernorm(first_tile_after(x_s[lo:lo + 16, :].astype(F32), anchor)).astype(BF16)
        return run

    def weight_jobs(dst, w_ref):
        n_rows, n_tiles = dst.shape[1] * 16, dst.shape[2]

        def job(r, j):
            def run(anchor):
                b11, b12, b21, b22 = (w_ref[pl.ds(a * n_rows + r, 16), pl.ds((b * n_tiles + j) * LANES, LANES)].astype(F32)
                                      for a in range(2) for b in range(2))
                b11, b22 = (jnp.concatenate([after(t[0:8], anchor), after(t[8:16], anchor)], axis=0)
                            for t in (b11, b22))
                for i, t in enumerate(_strassen_rhs(b11, b12, b21, b22)):
                    dst[i, r // 16, j] = t.astype(BF16)
            return run
        return [job(r, j) for r in range(0, n_rows, 16) for j in range(n_tiles)]

    def block_jobs(dst, signs, w_ref):
        n_rows, n_tiles = dst.shape[1] * 16, dst.shape[2]

        def job(r, j, products):
            def run(anchor):
                cols = signs.shape[2]
                tiles = {i: w_ref[pl.ds(i // cols * n_rows + r, 16), pl.ds((i % cols * n_tiles + j) * LANES, LANES)].astype(F32)
                         for i in np.flatnonzero(abs(signs[list(products)]).sum(axis=0)).tolist()}
                for t in products:
                    first = int(np.flatnonzero(signs[t])[0])
                    tied = jnp.concatenate([after(tiles[first][0:8], anchor), after(tiles[first][8:16], anchor)], axis=0)
                    terms = {i: tied if i == first else tiles[i] for i in np.flatnonzero(signs[t]).tolist()}
                    dst[t, r // 16, j] = _signed_sum(signs[t].ravel(), terms).astype(BF16)
            return run
        return [job(r, j, _share(range(len(signs)), part, 8))
                for r in range(0, n_rows, 16) for j in range(n_tiles) for part in range(8)]

    def project(a, w_ref, sums, order):
        lhs = _strassen_lhs(a[:, :FAST])
        fast, rest, products = _strassen_matmul(lambda i: lhs[i].astype(BF16), sums, order, dict(
            x=lambda: _dot(a[:, FAST:].astype(BF16), w_ref[FAST:, :]),
            y=lambda: _dot(a[:, :FAST].astype(BF16), w_ref[:FAST, FAST:])))
        return jnp.concatenate([fast, rest["y"]], axis=1) + rest["x"], products

    def normalize(lo, n):
        ln_s[lo:lo + n, :] = _layernorm(x_s[lo:lo + n, :].astype(F32)).astype(BF16)

    def project_k(lo, n, jobs=(), first=None, fast=False):
        if fast:
            k, parts = project(ln_s[lo:lo + n, :].astype(F32), wk_s, wk_x, QKV_ORDER)
        else:
            k = _dot(ln_s[lo:lo + n, :], wk_s[...] if first is None else wk_s[:, KA:])
            parts = [k]
        run_jobs(jobs, parts, 32)
        k = k.astype(BF16) if first is None else jnp.concatenate([first, k.astype(BF16)], axis=1)
        slabs = [pltpu.bitcast(k[:, j:j + LANES], U32) for j in range(0, D, LANES)]
        lane = lax.broadcasted_iota(jnp.int32, (n // 2, LANES), 1)
        for pair in range(NPAIR):
            j, off = divmod(pair * 2 * DH, LANES)
            kp = slabs[j]
            if off + 2 * DH > LANES:
                kp = jnp.where(lane >= LANES // 2, kp, slabs[j + 1])
            if off:
                kp = pltpu.roll(kp, LANES - off, 1)
            k_s[pair, lo // 2:(lo + n) // 2, :] = kp

    def project_qv(lo, n, fast, jobs=()):
        if fast:
            ln = ln_s[lo:lo + n, :].astype(F32)
            (q, q_parts), (v, v_parts) = project(ln, wq_s, wq_x, QKV_ORDER), project(ln, wv_s, wv_x, QKV_ORDER)
            run_jobs(jobs, q_parts + v_parts, 32)
        else:
            ln = ln_s[lo:lo + n, :]
            q, v = _dot(ln, wq_s[...]), _dot(ln, wv_s[...])
            run_jobs(jobs, [q, v], 32)
        q_s[:, lo:lo + n] = (q * q_scale).T
        vt = v.astype(BF16).astype(F32).T
        vmax = jnp.max(jnp.abs(vt).reshape(D // 8, 8, n), axis=0)
        row = lax.broadcasted_iota(jnp.int32, (8, n), 0)
        for j in range(n // CH):
            vmax_s[...] = jnp.maximum(vmax_s[...], vmax[:, j * CH:(j + 1) * CH])
        for pair in range(NPAIR):
            top = pair * 2 * DH
            mid = vt[top + 16:top + 24]
            both = jnp.concatenate([vt[top:top + 16], jnp.where(row < 4, mid, 1.0),
                                    jnp.where(row >= 4, mid, 1.0), vt[top + 24:top + 40]], axis=0)
            for j in range(n // CH):
                v_s[pair, lo // CH + j] = both[:, j * CH:(j + 1) * CH]

    cp_x0.wait()
    cp_wkb.start()
    normalize(0, RB)
    cp_wka.wait()
    cp_x1.start()
    cp_wq.start()
    cp_wv.start()
    cp_b2.wait()
    firsts = [_dot(ln_s[lo:lo + LANES, :], wk_s[:, :KA]).astype(BF16) for lo in range(0, RB, LANES)]
    cp_wkb.wait()
    cp_x2.start()
    cp_x1.wait()
    jobs = [norm_job(lo) for lo in range(RB, 2 * RB, 16)]
    for i, first in enumerate(firsts):
        project_k(i * LANES, LANES, _share(jobs, i, len(firsts)), first)
    for lo in range(RB, 2 * RB, LANES):
        project_k(lo, LANES)
    for cp in cp_late:
        cp.start()
    cp_wq.wait()
    cp_wv.wait()
    jobs = weight_jobs(wq_x, wq_s) + weight_jobs(wv_x, wv_s) + weight_jobs(wk_x, wk_s)
    project_qv(0, PB, False, jobs)
    cp_x2.wait()
    project_qv(PB, PB, True, [norm_job(lo) for lo in range(2 * RB, 3 * RB, 16)])
    for lo in range(2 * RB, S, PB):
        project_k(lo, PB, [norm_job(row) for row in range(lo + RB, min(lo + RB + PB, S), 16)], fast=True)
    for cp in cp_late:
        cp.wait()
    jobs = block_jobs(w1_x, WIDE_K[1], w1_s) + block_jobs(w2_x, WIDE_N[1], w2_s) + weight_jobs(wo_x, wo_s)
    blocks = range(2 * PB, S, PB)
    for i, lo in enumerate(blocks):
        project_qv(lo, PB, True, _share(jobs, i, len(blocks)))

    p_words = p_s.bitcast(U32)
    qrow = lax.broadcasted_iota(jnp.int32, (8, NQ), 0)

    def q_rows(pair, lo, n):
        start = pair * 2 * DH + lo
        return pl.ds(start if isinstance(start, int) else pl.multiple_of(start, 8), n)

    def head_rows(odd):
        return pl.ds(odd * HROWS, HROWS)

    def q_weights(pair, odd, qb):
        cols = rows_of(qb, NQ)
        mid = q_s[q_rows(pair, 16, 8), cols]
        zero = jnp.zeros((8, NQ), F32)
        if odd:
            parts = [zero, zero, jnp.where(qrow >= 4, mid, 0.0), q_s[q_rows(pair, 24, 16), cols], zero]
        else:
            parts = [q_s[q_rows(pair, 0, 16), cols], jnp.where(qrow < 4, mid, 0.0), zero]
        return jnp.concatenate(parts, axis=0).astype(BF16)

    def spread_k(z, pair, odd, c, dims, anchor=None):
        k = k_s[pair, ((c + 1) * CH - NV) // 2:(c + 1) * CH // 2, :]
        if anchor is not None:
            k = after(k, anchor)
        k = pltpu.bitcast(k, BF16).astype(F32)
        for d in dims:
            kb_s[z, odd, c, d] = jnp.broadcast_to(k[:, odd * DH + d:odd * DH + d + 1], (NV, LANES))

    def spread_q(z, pair, odd, qb, dims, anchor=None):
        for d in dims:
            r = odd * DH + d
            q = q_s[q_rows(pair, r // 8 * 8, 8), rows_of(qb, NQ)]
            if anchor is not None:
                q = jnp.concatenate([after(q[:, j:j + LANES], anchor) for j in range(0, NQ, LANES)], axis=1)
            qb_s[z, qb, d] = jnp.broadcast_to(q[r % 8:r % 8 + 1, :], (8, NQ))

    def vector_probs(z, odd, qb, c, keys=None):
        s = None
        for piece in range(len(KEY_MARKS) + 1):
            for d in _share(range(DH), piece, len(KEY_MARKS) + 1):
                t = (jnp.concatenate([kb_s[z, odd, c, d]] * NT, axis=1)
                     * jnp.concatenate([qb_s[z, qb, d]] * (NV // 8), axis=0))
                s = t if s is None else s + t
            if keys is not None and piece < len(KEY_MARKS):
                for r in range(0, NV, 8):
                    for j in range(0, NQ, LANES):
                        keys[KEY_MARKS[piece]] = after(keys[KEY_MARKS[piece]], s[r:r + 8, j:j + LANES])
        return jnp.exp2(s).astype(BF16)

    def key_tiles(pair, c):
        return [k_s[pair, (c * CH + i) // 2:(c * CH + i) // 2 + 8, :] for i in range(0, CH - NV, 16)]

    def mxu_scores(keys, q):
        k = pltpu.bitcast(jnp.concatenate(keys, axis=0), BF16)
        return _dot(k[:, :q.shape[0]], q)

    def store_probs(z, slot, c, s):
        p = jnp.exp2(s)
        for i in range((CH - NV) // 16):
            for j in range(NT):
                p_s[z, slot, c, i, j] = p[16 * i:16 * (i + 1), j * LANES:(j + 1) * LANES].astype(BF16)

    def attention_rows(r):
        row = lax.broadcasted_iota(jnp.int32, (8, FB), 0)
        parts = []
        for pair in range(NPAIR):
            acc = o_s[pair, :, rows_of(r, FB)]
            inv_even, inv_odd = 1.0 / acc[DH:DH + 1], 1.0 / acc[HROWS:HROWS + 1]
            parts += [acc[0:16] * inv_even, jnp.where(row < 4, acc[16:24] * inv_even, acc[24:32] * inv_odd),
                      acc[32:48] * inv_odd]
        return jnp.concatenate(parts, axis=0).T

    def residual_norm(r, proj):
        rows = rows_of(r, FB)
        hid = x_s[rows, :].astype(F32) + proj
        h_s[rows, :] = hid
        ln = _layernorm(hid)
        for i, a in enumerate(_operands(WIDE_K[0], ln)):
            lnx_s[r % 2, i] = a.astype(BF16)

    for c in range(NC):
        spread_k(0, 0, 0, c, range(DH))
    for qb in range(NQB):
        spread_q(0, 0, 0, qb, range(DH))
    q_first = q_weights(0, 0, 0)
    for c in range(NC):
        store_probs(0, 0, c, mxu_scores(key_tiles(0, c), q_first))
    pv_s[...] = vector_probs(0, 0, 0, 0)
    range_s[...] = jnp.ones(range_s.shape, F32)

    def head(pair, odd, final=False):
        p_vec, sum_lo, sum_hi = pv_s[...], range_s[odd, 0], range_s[odd, 1]
        z = zero_s[0]
        for qb in range(NQB):
            ahead = (pair, odd, qb + 1) if qb + 1 < NQB else (pair + odd, 1 - odd, 0)
            drain = final and qb + 1 == NQB
            if drain:
                o_first = attention_rows(0).astype(BF16)
            else:
                q = q_weights(*ahead)
            for c in range(NC):
                keys = None if drain else key_tiles(ahead[0], c)
                if c + 1 < NC:
                    p_next = vector_probs(z, odd, qb, c + 1, keys)
                elif not drain:
                    p_next = vector_probs(z, ahead[1], ahead[2], 0, keys)
                if not drain:
                    s = mxu_scores(keys, q)
                elif 0 <= c - 3 < D // LANES:
                    j = (c - 3) * LANES
                    part = _dot(o_first[:, j:j + LANES], wo_s[j:j + LANES, :])
                    proj = part if j == 0 else part + proj
                    if j + LANES == D:
                        residual_norm(0, proj)
                p = jnp.concatenate(
                    [jnp.concatenate([pltpu.bitcast(p_words[z, qb % 2, c, i, j], BF16) for j in range(NT)], axis=1)
                     for i in range((CH - NV) // 16)] + [p_vec], axis=0)
                o = _dot(v_s[pair, c, head_rows(odd), :], p)
                acc = o if c == 0 else o + acc
                p_vec = p_next
                if drain:
                    continue
                store_probs(z, (qb + 1) % 2, c, s)
                anchor = s[0:8, 0:LANES]
                group, part_of = divmod(qb * NC + c, NQB)
                if not final:
                    spread_k(z, pair + odd, 1 - odd, group, _share(range(DH), part_of, NQB), anchor)
                if 0 <= c - 5 < 10:
                    dims = _share(range(DH), c - 5, 10)
                    if qb == 0:
                        spread_q(z, pair, odd, NQB - 1, dims, anchor)
                    elif not final:
                        spread_q(z, pair + odd, 1 - odd, qb - 1, dims, anchor)
            o_s[pair, head_rows(odd), rows_of(qb, NQ)] = acc
            sums = acc[0:8] if odd else acc[16:24]
            sum_lo, sum_hi = jnp.minimum(sum_lo, sums), jnp.maximum(sum_hi, sums)
        pv_s[...] = p_vec
        range_s[odd, 0], range_s[odd, 1] = sum_lo, sum_hi

    def head_step(h, _):
        for odd in range(2):
            pl.when(h % 2 == odd)(functools.partial(head, h // 2, odd))
        return 0

    lax.fori_loop(0, NUM_HEADS - 1, head_step, 0)
    head(NPAIR - 1, 1, final=True)

    sum_lo = jnp.where(qrow >= 4, range_s[0, 0], range_s[1, 0])
    sum_hi = jnp.where(qrow >= 4, range_s[0, 1], range_s[1, 1])
    flags = jnp.where((sum_lo >= SUM_LO) & (sum_hi <= SUM_HI), 0.0, 1.0)
    unsafe = jnp.max(functools.reduce(jnp.maximum, [flags[:, j:j + LANES] for j in range(0, NQ, LANES)],
                                      jnp.where(vmax_s[...] <= VALUE_HI, 0.0, 1.0)))

    @pl.when(unsafe > 0.0)
    def _():
        def exact(i, _):
            pair, qb = i // NQB, i % NQB
            k = pltpu.bitcast(k_s[pair], BF16)
            for odd in range(2):
                q = q_weights(pair, odd, qb)
                s = _dot(k[:, :q.shape[0]], q)
                p = jnp.exp2(s - jnp.max(s, axis=0, keepdims=True)).astype(BF16)
                v = jnp.concatenate([v_s[pair, c, head_rows(odd), :] for c in range(NC)], axis=1)
                o_s[pair, head_rows(odd), rows_of(qb, NQ)] = _dot(v, p)
            return 0

        lax.fori_loop(0, NPAIR * NQB, exact, 0)
        residual_norm(0, _dot(attention_rows(0).astype(BF16), wo_s[...]))

    b1 = b1_s[...].astype(F32).reshape(1, -1)
    b2 = b2_s[...].astype(F32).reshape(1, -1)

    def project_out(r):
        residual_norm(r, project(attention_rows(r), wo_s, wo_x, WO_ORDER)[0])

    def ffn(r, orders, meanwhile=lambda: None):
        rows = rows_of(r, FB)
        lhs = [lnx_s[r % 2, t] for t in range(len(_SCHEME))]
        up, down = ([ord(c) - ord("a") for c in order] for order in orders)
        hidden = _fast_matmul(WIDE_K, lambda t: lhs[t], w1_x, up, [(PROJECT_AT, meanwhile)])
        lhs = _operands(WIDE_N[0], jnp.square(jnp.maximum(hidden + b1, 0.0)))
        y = _fast_matmul(WIDE_N, lambda t: lhs[t].astype(BF16), w2_x, down, [(PROJECT_AT - len(up), meanwhile)])
        out_s[rows, :] = (h_s[rows, :] + (y + b2)).astype(out_s.dtype)

    def write_back(r):
        return pltpu.make_async_copy(out_s.at[rows_of(r, FB), :], out_hbm.at[0, rows_of(r, FB), :], out_sem.at[r])

    def block_step(r, _):
        ffn(r, FFN_ORDER, lambda: project_out(r + 1))
        write_back(r).start()
        return 0

    n_blocks = S // FB
    lax.fori_loop(0, n_blocks - 1, block_step, 0)
    ffn(n_blocks - 1, LAST_FFN_ORDER)
    write_back(n_blocks - 1).start()
    for r in range(n_blocks):
        write_back(r).wait()


@jax.jit
def pallas_sequential_preLN__softmax_full_mha__dense_activation_squared_relu__prompt_kernel(
    A_x: jax.Array,
    A_wqkv: jax.Array,
    A_wo: jax.Array,
    B_x: jax.Array,
    B_w1: jax.Array,
    B_b1: jax.Array,
    B_w2: jax.Array,
    B_b2: jax.Array,
):
    del B_x
    _, S, D = A_x.shape
    F = B_w1.shape[1]
    pairs, dh = NUM_HEADS // 2, D // NUM_HEADS
    vmem = pltpu.VMEM
    scratch = [
        vmem((S, D), A_x.dtype),
        vmem((D, D), A_wqkv.dtype), vmem((D, D), A_wqkv.dtype), vmem((D, D), A_wqkv.dtype),
        vmem(A_wo.shape, A_wo.dtype),
        vmem(B_w1.shape, B_w1.dtype), vmem(B_b1.shape, B_b1.dtype),
        vmem(B_w2.shape, B_w2.dtype), vmem(B_b2.shape, B_b2.dtype),
        *[vmem((7, FAST // 32, FAST // 2 // LANES, 16, LANES), BF16)] * 4,
        vmem((len(_SCHEME), LANES // 16, F // 3 // LANES, 16, LANES), BF16),
        vmem((len(_SCHEME), F // 3 // 16, 1, 16, LANES), BF16),
        vmem((S, D), BF16),
        vmem((2, len(_SCHEME), FB // 2, LANES), BF16),
        vmem((S, D), F32),
        vmem((S, D), A_x.dtype),
        vmem((pairs, S // 2, LANES), U32),
        vmem((D, S), F32),
        vmem((pairs, S // CH, 2 * HROWS, CH), F32),
        vmem((1, 2, S // CH, (CH - NV) // 16, NQ // LANES, 16, LANES), BF16),
        vmem((1, 2, S // CH, dh, NV, LANES), F32),
        vmem((1, S // NQ, dh, 8, NQ), F32),
        vmem((NV, NQ), BF16),
        vmem((pairs, 2 * HROWS, S), F32),
        vmem((2, 2, 8, NQ), F32),
        vmem((8, CH), F32),
        vmem((8, LANES), jnp.int32),
        pltpu.SMEM((1,), jnp.int32),
        pltpu.SemaphoreType.DMA((12,)),
        pltpu.SemaphoreType.DMA((S // FB,)),
    ]
    hbm = pl.BlockSpec(memory_space=pl.ANY)
    return pl.pallas_call(
        _kernel,
        out_shape=jax.ShapeDtypeStruct(A_x.shape, A_x.dtype),
        in_specs=[hbm] * 7,
        out_specs=hbm,
        scratch_shapes=scratch,
        compiler_params=pltpu.CompilerParams(vmem_limit_bytes=100 * 2 ** 20),
    )(A_x, A_wqkv, A_wo, B_w1, B_b1, B_w2, B_b2)
```
